```python
import os as _os
_os.environ.setdefault("JAX_PLATFORMS", "cpu")
import jax
import jax.numpy as jnp

def _softmax(x, axis=-1):
    return jax.nn.softmax(x, axis=axis)
def _gelu(x):
    return jax.nn.gelu(x, approximate=True)
def _silu(x):
    return jax.nn.silu(x)
def _sigmoid(x):
    return jax.nn.sigmoid(x)
def _layernorm(x, axis=-1, eps=1e-5):
    m = jnp.mean(x, axis=axis, keepdims=True)
    v = jnp.var(x, axis=axis, keepdims=True)
    return (x - m) / jnp.sqrt(v + eps)
def _scatter_add(tgt, idx, src, axis=0):
    return tgt.at[idx].add(src)
def _segment_sum(src, seg, n):
    return jax.ops.segment_sum(src, seg, n)
class _Rng:
    def __init__(self, key):
        self._k = key
    def _next(self):
        self._k, sub = jax.random.split(self._k)
        return sub
    def normal(self, shape):
        return jax.random.normal(self._next(), shape, dtype=jnp.bfloat16)
    def randint(self, lo, hi, shape):
        return jax.random.randint(self._next(), shape, lo, hi, dtype=jnp.int32)
    def uniform(self, shape, lo=0.0, hi=1.0):
        return jax.random.uniform(self._next(), shape, jnp.bfloat16, lo, hi)
    def permutation(self, n):
        return jax.random.permutation(self._next(), n)


kernel_name = 'standalone__gqa_block_cached__sampling'

def setup_inputs():
    _rng = _Rng(jax.random.key(int.from_bytes(__import__("os").urandom(4), "little")))
    _w = (lambda a: (lambda t: t.astype(jnp.bfloat16) if jnp.issubdtype(t.dtype, jnp.floating) else t)(jnp.asarray(a)))
    B, Sq, D = 32, 16, 1024
    Hq, Hkv, Sk, Dh = 32, 4, 2048, 128
    assert Hq % Hkv == 0, (Hq, Hkv)
    return {
        "x": _w((lambda *s: _rng.normal(s) * 0.8)(B, Sq, D)),
        "k_cache": _w((lambda *s: _rng.normal(s) * 0.8)(B, Hkv, Sk, Dh)),
        "v_cache": _w((lambda *s: _rng.normal(s) * 0.05)(B, Hkv, Sk, Dh)),
        "wq": _w((lambda *s: _rng.normal(s) * 0.8)(D, Hq * Dh) * (D ** -0.5)),
        "wo": _w((lambda *s: _rng.normal(s) * 0.05)(Hq * Dh, D) * ((Hq * Dh) ** -0.5)),
    }

def reference(x, k_cache, v_cache, wq, wo):
    B, Sq, D = x.shape
    Hq, Dh = 32, 128
    Hkv = k_cache.shape[1]
    rep = Hq // Hkv
    q = (lambda x, *d: x.transpose(*d))((x @ wq).reshape(B, Sq, Hq, Dh), 0, 2, 1, 3)
    k = jnp.repeat(k_cache, rep, axis=1)
    v = jnp.repeat(v_cache, rep, axis=1)
    scores = jnp.einsum("bhqd,bhkd->bhqk", q, k) * (Dh ** -0.5)
    p = _softmax(scores, axis=-1)
    o = jnp.einsum("bhqk,bhkd->bhqd", p, v)
    return (lambda x, *d: x.transpose(*d))(o, 0, 2, 1, 3).reshape(B, Sq, Hq * Dh) @ wo
```

```python
import functools, math
import jax, jax.numpy as jnp
import jax.experimental.pallas as pl
import jax.experimental.pallas.tpu as pltpu

B, Sq, D = 32, 16, 1024
Hq, Hkv, Sk, Dh = 32, 4, 2048, 128
REP = Hq // Hkv
G = REP * Dh
QSCALE = (Dh ** -0.5) * math.log2(math.e)
NSLOT = 8
NPROB = B * Hkv

def kernel(x_hbm, k_hbm, v_hbm, wq_hbm, wo_hbm, out_ref,
           x_v, wq_v, wo_v, kbuf, vbuf, q_s, o_s, acc_s,
           sem_x, sem_wq, sem_wo, sem_k, sem_v):

    def kv_copies(i, slot):
        h = i // B
        b = i % B
        return (pltpu.make_async_copy(k_hbm.at[b, h], kbuf.at[slot], sem_k.at[slot]),
                pltpu.make_async_copy(v_hbm.at[b, h], vbuf.at[slot], sem_v.at[slot]))

    def wq_copy(h):
        return pltpu.make_async_copy(wq_hbm.at[:, pl.ds(h * G, G)], wq_v, sem_wq)

    def wo_copy(h):
        return pltpu.make_async_copy(wo_hbm.at[pl.ds(h * G, G), :], wo_v, sem_wo)

    x_copy = pltpu.make_async_copy(x_hbm, x_v, sem_x)

    x_copy.start()
    wq_copy(0).start()
    for s in range(2):
        for c in kv_copies(s, s):
            c.start()
    x_copy.wait()
    wq_copy(0).wait()
    for s in range(2, NSLOT):
        for c in kv_copies(s, s):
            c.start()
    wo_copy(0).start()

    def body(i, carry):
        h = i // B
        b = i % B
        slot = i % NSLOT

        @pl.when(b == 0)
        def _():
            @pl.when(h > 0)
            def _():
                wq_copy(h).wait()
            q = jnp.dot(x_v[...], wq_v[...], preferred_element_type=jnp.float32) * QSCALE
            q = q.astype(jnp.bfloat16)
            for r in range(REP):
                q_s[:, r * Sq:(r + 1) * Sq, :] = q[:, r * Dh:(r + 1) * Dh].reshape(B, Sq, Dh)
            @pl.when(h + 1 < Hkv)
            def _():
                wq_copy(h + 1).start()

        for c in kv_copies(i, slot):
            c.wait()
        q = q_s[b]
        k = kbuf[slot]
        v = vbuf[slot]
        s = jax.lax.dot_general(q, k, (((1,), (1,)), ((), ())), preferred_element_type=jnp.float32)
        m = jnp.max(s, axis=-1, keepdims=True)
        p = jnp.exp2(s - m)
        l = jnp.sum(p, axis=-1, keepdims=True)
        o = jnp.dot(p.astype(jnp.bfloat16), v, preferred_element_type=jnp.float32)
        o = (o / l).astype(jnp.bfloat16)
        row = pl.multiple_of(b * Sq, Sq)
        for r in range(REP):
            o_s[pl.ds(row, Sq), r * Dh:(r + 1) * Dh] = o[r * Sq:(r + 1) * Sq, :]

        @pl.when(i + NSLOT < NPROB)
        def _():
            for c in kv_copies(i + NSLOT, slot):
                c.start()

        @pl.when(b == B - 1)
        def _():
            wo_copy(h).wait()
            contrib = jnp.dot(o_s[...], wo_v[...], preferred_element_type=jnp.float32)
            @pl.when(h == 0)
            def _():
                acc_s[...] = contrib
            @pl.when(h > 0)
            def _():
                acc_s[...] += contrib
            @pl.when(h + 1 < Hkv)
            def _():
                wo_copy(h + 1).start()
        return carry

    jax.lax.fori_loop(0, NPROB, body, 0)
    out_ref[...] = acc_s[...].astype(out_ref.dtype)

@jax.jit
def pallas_standalone__gqa_block_cached__sampling_kernel(x, k_cache, v_cache, wq, wo):
    x2 = x.reshape(B * Sq, D)
    anyspec = pl.BlockSpec(memory_space=pl.ANY)
    out = pl.pallas_call(
        kernel,
        in_specs=[anyspec] * 5,
        out_specs=pl.BlockSpec((B * Sq, D), lambda: (0, 0)),
        out_shape=jax.ShapeDtypeStruct((B * Sq, D), jnp.bfloat16),
        scratch_shapes=[
            pltpu.VMEM((B * Sq, D), jnp.bfloat16),
            pltpu.VMEM((D, G), jnp.bfloat16),
            pltpu.VMEM((G, D), jnp.bfloat16),
            pltpu.VMEM((NSLOT, Sk, Dh), jnp.bfloat16),
            pltpu.VMEM((NSLOT, Sk, Dh), jnp.bfloat16),
            pltpu.VMEM((B, REP * Sq, Dh), jnp.bfloat16),
            pltpu.VMEM((B * Sq, G), jnp.bfloat16),
            pltpu.VMEM((B * Sq, D), jnp.float32),
            pltpu.SemaphoreType.DMA(()),
            pltpu.SemaphoreType.DMA(()),
            pltpu.SemaphoreType.DMA(()),
            pltpu.SemaphoreType.DMA((NSLOT,)),
            pltpu.SemaphoreType.DMA((NSLOT,)),
        ],
        compiler_params=pltpu.CompilerParams(vmem_limit_bytes=100 * 1024 * 1024),
    )(x2, k_cache, v_cache, wq, wo)
    return out.reshape(B, Sq, D)
```

```python
import functools, math
import jax, jax.numpy as jnp
import jax.experimental.pallas as pl
import jax.experimental.pallas.tpu as pltpu

B, Sq, D = 32, 16, 1024
Hq, Hkv, Sk, Dh = 32, 4, 2048, 128
REP = Hq // Hkv
G = REP * Dh
QSCALE = (Dh ** -0.5) * math.log2(math.e)
NSLOT = 8
NPROB = B * Hkv
GB = 8
NG = B // GB
GR = GB * Sq

def kernel(x_hbm, k_hbm, v_hbm, wq_hbm, wo_hbm, out_hbm,
           x_v, wq_v, wo_v, kbuf, vbuf, q_s, o_s, acc_s, obuf,
           sem_x, sem_wq, sem_wo, sem_k, sem_v, sem_o):

    def kv_copies(i, slot):
        h = i // B
        b = i % B
        return (pltpu.make_async_copy(k_hbm.at[b, h], kbuf.at[slot], sem_k.at[slot]),
                pltpu.make_async_copy(v_hbm.at[b, h], vbuf.at[slot], sem_v.at[slot]))

    def wq_copy(h):
        return pltpu.make_async_copy(wq_hbm.at[:, pl.ds(h * G, G)], wq_v, sem_wq)

    def wo_copy(h):
        return pltpu.make_async_copy(wo_hbm.at[pl.ds(h * G, G), :], wo_v, sem_wo)

    def out_copy(g):
        rows = pl.ds(pl.multiple_of(g * GR, GR), GR)
        return pltpu.make_async_copy(obuf.at[rows, :], out_hbm.at[rows, :], sem_o.at[g])

    def tail_copy(j):
        n = (GB - 1) * Sq
        base = (NG - 1) * GR
        rows = pl.ds(base, n) if j == 0 else pl.ds(base + n, Sq)
        return pltpu.make_async_copy(obuf.at[rows, :], out_hbm.at[rows, :], sem_o.at[NG - 1 + j])

    x_copy = pltpu.make_async_copy(x_hbm, x_v, sem_x)

    x_copy.start()
    wq_copy(0).start()
    for s in range(2):
        for c in kv_copies(s, s):
            c.start()
    x_copy.wait()
    wq_copy(0).wait()
    for s in range(2, NSLOT):
        for c in kv_copies(s, s):
            c.start()
    wo_copy(0).start()

    def body(i, carry):
        h = i // B
        b = i % B
        slot = i % NSLOT
        g = b // GB
        grow = pl.multiple_of(g * GR, GR)

        @pl.when(b % GB == 0)
        def _():
            @pl.when(jnp.logical_and(h > 0, b == 0))
            def _():
                wq_copy(h).wait()
            q = jnp.dot(x_v[pl.ds(grow, GR), :], wq_v[...], preferred_element_type=jnp.float32) * QSCALE
            q = q.astype(jnp.bfloat16)
            for r in range(REP):
                q_s[:, r * Sq:(r + 1) * Sq, :] = q[:, r * Dh:(r + 1) * Dh].reshape(GB, Sq, Dh)
            @pl.when(jnp.logical_and(h + 1 < Hkv, g == NG - 1))
            def _():
                wq_copy(h + 1).start()

        for c in kv_copies(i, slot):
            c.wait()
        q = q_s[b % GB]
        k = kbuf[slot]
        v = vbuf[slot]
        s = jax.lax.dot_general(q, k, (((1,), (1,)), ((), ())), preferred_element_type=jnp.float32)
        m = jnp.max(s, axis=-1, keepdims=True)
        p = jnp.exp2(s - m)
        l = jnp.sum(p, axis=-1, keepdims=True)
        o = jnp.dot(p.astype(jnp.bfloat16), v, preferred_element_type=jnp.float32)
        o = (o / l).astype(jnp.bfloat16)
        row = pl.multiple_of((b % GB) * Sq, Sq)
        for r in range(REP):
            o_s[pl.ds(row, Sq), r * Dh:(r + 1) * Dh] = o[r * Sq:(r + 1) * Sq, :]

        @pl.when(i + NSLOT < NPROB)
        def _():
            for c in kv_copies(i + NSLOT, slot):
                c.start()

        last_group = jnp.logical_and(h == Hkv - 1, g == NG - 1)

        @pl.when(jnp.logical_and(b % GB == GB - 1, jnp.logical_not(last_group)))
        def _():
            @pl.when(g == 0)
            def _():
                wo_copy(h).wait()
            contrib = jnp.dot(o_s[...], wo_v[...], preferred_element_type=jnp.float32)
            @pl.when(h == 0)
            def _():
                acc_s[pl.ds(grow, GR), :] = contrib
            @pl.when(jnp.logical_and(h > 0, h < Hkv - 1))
            def _():
                acc_s[pl.ds(grow, GR), :] += contrib
            @pl.when(h == Hkv - 1)
            def _():
                obuf[pl.ds(grow, GR), :] = (acc_s[pl.ds(grow, GR), :] + contrib).astype(obuf.dtype)
                out_copy(g).start()
            @pl.when(jnp.logical_and(h + 1 < Hkv, g == NG - 1))
            def _():
                wo_copy(h + 1).start()

        @pl.when(i == NPROB - 2)
        def _():
            n = (GB - 1) * Sq
            base = (NG - 1) * GR
            contrib = jnp.dot(o_s[0:n, :], wo_v[...], preferred_element_type=jnp.float32)
            obuf[base:base + n, :] = (acc_s[base:base + n, :] + contrib).astype(obuf.dtype)
            tail_copy(0).start()

        @pl.when(i == NPROB - 1)
        def _():
            n = (GB - 1) * Sq
            base = (NG - 1) * GR
            contrib = jnp.dot(o_s[n:, :], wo_v[...], preferred_element_type=jnp.float32)
            obuf[base + n:, :] = (acc_s[base + n:, :] + contrib).astype(obuf.dtype)
            tail_copy(1).start()
        return carry

    jax.lax.fori_loop(0, NPROB, body, 0)
    for g in range(NG - 1):
        out_copy(g).wait()
    tail_copy(0).wait()
    tail_copy(1).wait()

@jax.jit
def pallas_standalone__gqa_block_cached__sampling_kernel(x, k_cache, v_cache, wq, wo):
    x2 = x.reshape(B * Sq, D)
    anyspec = pl.BlockSpec(memory_space=pl.ANY)
    out = pl.pallas_call(
        kernel,
        in_specs=[anyspec] * 5,
        out_specs=anyspec,
        out_shape=jax.ShapeDtypeStruct((B * Sq, D), jnp.bfloat16),
        scratch_shapes=[
            pltpu.VMEM((B * Sq, D), jnp.bfloat16),
            pltpu.VMEM((D, G), jnp.bfloat16),
            pltpu.VMEM((G, D), jnp.bfloat16),
            pltpu.VMEM((NSLOT, Sk, Dh), jnp.bfloat16),
            pltpu.VMEM((NSLOT, Sk, Dh), jnp.bfloat16),
            pltpu.VMEM((GB, REP * Sq, Dh), jnp.bfloat16),
            pltpu.VMEM((GR, G), jnp.bfloat16),
            pltpu.VMEM((B * Sq, D), jnp.float32),
            pltpu.VMEM((B * Sq, D), jnp.bfloat16),
            pltpu.SemaphoreType.DMA(()),
            pltpu.SemaphoreType.DMA(()),
            pltpu.SemaphoreType.DMA(()),
            pltpu.SemaphoreType.DMA((NSLOT,)),
            pltpu.SemaphoreType.DMA((NSLOT,)),
            pltpu.SemaphoreType.DMA((NG + 1,)),
        ],
        compiler_params=pltpu.CompilerParams(vmem_limit_bytes=100 * 1024 * 1024),
    )(x2, k_cache, v_cache, wq, wo)
    return out.reshape(B, Sq, D)
```
